```python
import os as _os
_os.environ.setdefault("JAX_PLATFORMS", "cpu")
import jax
import jax.numpy as jnp

def _softmax(x, axis=-1):
    return jax.nn.softmax(x, axis=axis)
def _gelu(x):
    return jax.nn.gelu(x, approximate=True)
def _silu(x):
    return jax.nn.silu(x)
def _sigmoid(x):
    return jax.nn.sigmoid(x)
def _layernorm(x, axis=-1, eps=1e-5):
    m = jnp.mean(x, axis=axis, keepdims=True)
    v = jnp.var(x, axis=axis, keepdims=True)
    return (x - m) / jnp.sqrt(v + eps)
def _scatter_add(tgt, idx, src, axis=0):
    return tgt.at[idx].add(src)
def _segment_sum(src, seg, n):
    return jax.ops.segment_sum(src, seg, n)
class _Rng:
    def __init__(self, key):
        self._k = key
    def _next(self):
        self._k, sub = jax.random.split(self._k)
        return sub
    def normal(self, shape):
        return jax.random.normal(self._next(), shape, dtype=jnp.bfloat16)
    def randint(self, lo, hi, shape):
        return jax.random.randint(self._next(), shape, lo, hi, dtype=jnp.int32)
    def uniform(self, shape, lo=0.0, hi=1.0):
        return jax.random.uniform(self._next(), shape, jnp.bfloat16, lo, hi)
    def permutation(self, n):
        return jax.random.permutation(self._next(), n)


kernel_name = 'gated_mix__softmax_full_mha__dense_activation_relu__prompt'

def setup_inputs():
    _rng = _Rng(jax.random.key(int.from_bytes(__import__("os").urandom(4), "little")))
    _w = (lambda a: (lambda t: t.astype(jnp.bfloat16) if jnp.issubdtype(t.dtype, jnp.floating) else t)(jnp.asarray(a)))
    def _A_setup():
        B, S, D = 1, 2048, 640
        return {
            "x": _w((lambda *s: _rng.normal(s) * 0.05)(B, S, D)),
            "wqkv": _w((lambda *s: _rng.normal(s) * 0.8)(D, 3 * D)),
            "wo": _w((lambda *s: _rng.normal(s) * 0.05)(D, D)),
        }
    _A_in = _A_setup()

    def _B_setup():
        B, S, D, Dff = 1, 2048, 640, 1536
        return {
            "x": _w((lambda *s: _rng.normal(s) * 0.05)(B, S, D)),
            "w1": _w((lambda *s: _rng.normal(s) * 0.05)(D, Dff)),
            "w2": _w((lambda *s: _rng.normal(s) * 0.05)(Dff, D)),
        }
    _B_in = _B_setup()

    return {
        "A_x": _A_in["x"],
        "A_wqkv": _A_in["wqkv"],
        "A_wo": _A_in["wo"],
        "B_x": _B_in["x"],
        "B_w1": _B_in["w1"],
        "B_w2": _B_in["w2"],
        "gate_w": _w((lambda *s: _rng.normal(s) * 0.05)(640) * 16.0),
    }

def reference(A_x, A_wqkv, A_wo, B_x, B_w1, B_w2, gate_w):
    def _A_ref(x, wqkv, wo):
        B, S, D = x.shape
        H = 32; Dh = D // H
        qkv = (lambda x, *d: x.transpose(*d))((x @ wqkv).reshape(B, S, 3, H, Dh), 2, 0, 3, 1, 4)
        q, k, v = qkv[0], qkv[1], qkv[2]
        scale = Dh ** -0.5
        scores = jnp.einsum("bhqd,bhkd->bhqk", q, k) * scale
        p = _softmax(scores, axis=-1)
        o = jnp.einsum("bhqk,bhkd->bhqd", p, v)
        return (lambda x, *d: x.transpose(*d))(o, 0, 2, 1, 3).reshape(B, S, D) @ wo

    def _B_ref(x, w1, w2):
        h = jnp.einsum("bsd,df->bsf", x, w1)
        zero = jnp.zeros_like(h)
        h = jnp.maximum(h, zero)
        return jnp.einsum("bsf,fd->bsd", h, w2)

    x = A_x
    g = _sigmoid((x * gate_w).sum(-1, keepdims=True))
    a = _A_ref(x, A_wqkv, A_wo)
    b = _B_ref(x, B_w1, B_w2)
    return g * a + (1 - g) * b
```

```python
import functools
import math

import jax
import jax.numpy as jnp
import jax.experimental.pallas as pl
import jax.experimental.pallas.tpu as pltpu

S, D, H, DH, DFF = 2048, 640, 32, 20, 1536
NPAIR = H // 2
NWIN = 9
TQ = 256
NQ = S // TQ
TS = 512
TK = 512
F32 = jnp.float32
BF16 = jnp.bfloat16
QSCALE = (DH ** -0.5) * math.log2(math.e)


def _kernel(x_ref, wqkv_ref, wo_ref, w1_ref, w2_ref, gw_ref, o_ref,
            k_scr, qt_scr, vt_scr, s_scr, m_scr, ot_scr):
    i = pl.program_id(0)

    def masked_qt(qi, pj):
        w = jnp.minimum((40 * pj) // 64, NWIN - 1)
        qt = qt_scr[qi, w]
        row = jax.lax.broadcasted_iota(jnp.int32, (128, TQ), 0)
        rel = (row - 40 * pj) & 127
        zero = jnp.zeros_like(qt)
        qe = jnp.where(rel < DH, qt, zero)
        qo = jnp.where(jnp.logical_and(rel >= DH, rel < 2 * DH), qt, zero)
        return w, jnp.concatenate([qe, qo], axis=1)

    def scores_chunk(w, qtm, c):
        s = jnp.dot(k_scr[w, pl.ds(c * TK, TK), :], qtm,
                    preferred_element_type=F32)
        s_scr[pl.ds(c * TK, TK), :] = s
        return jnp.max(s.reshape(TK // 8, 8, 2 * TQ), axis=0)

    def finish_max(mx):
        m_scr[...] = jnp.broadcast_to(jnp.max(mx, axis=0, keepdims=True),
                                      (8, 2 * TQ))

    @pl.when(i == 0)
    def _projections():
        lane = jax.lax.broadcasted_iota(jnp.int32, (TS, 128), 1)
        sub = jax.lax.broadcasted_iota(jnp.int32, (8, TS), 0)
        ones = jnp.ones((8, TS), F32)
        for r in range(S // TS):
            xs = x_ref[pl.ds(r * TS, TS), :]
            q = jnp.dot(xs, wqkv_ref[:, pl.ds(0, D)],
                        preferred_element_type=F32) * QSCALE
            qt = q.T.astype(BF16)
            for u in range(TS // TQ):
                qi = r * (TS // TQ) + u
                cols = qt[:, u * TQ:(u + 1) * TQ]
                for g in range(5):
                    qt_scr[qi, 2 * g] = cols[128 * g:128 * g + 128]
                for g in range(4):
                    qt_scr[qi, 2 * g + 1, pl.ds(0, 64), :] = (
                        cols[128 * (g + 1):128 * (g + 1) + 64])
                    qt_scr[qi, 2 * g + 1, pl.ds(64, 64), :] = (
                        cols[128 * g + 64:128 * g + 128])
            k = jnp.dot(xs, wqkv_ref[:, pl.ds(D, D)],
                        preferred_element_type=F32)
            for g in range(5):
                k_scr[2 * g, pl.ds(r * TS, TS), :] = (
                    k[:, 128 * g:128 * g + 128].astype(BF16))
            for g in range(4):
                k_scr[2 * g + 1, pl.ds(r * TS, TS), :] = jnp.where(
                    lane >= 64, k[:, 128 * g:128 * g + 128],
                    k[:, 128 * (g + 1):128 * (g + 1) + 128]).astype(BF16)
            v = jnp.dot(xs, wqkv_ref[:, pl.ds(2 * D, D)],
                        preferred_element_type=F32)
            vt = v.astype(BF16).astype(F32).T
            for j in range(NPAIR):
                b = 40 * j
                mid = vt[b + 16:b + 24]
                vt_scr[2 * j, pl.ds(0, 16), pl.ds(r * TS, TS)] = vt[b:b + 16]
                vt_scr[2 * j, pl.ds(16, 8), pl.ds(r * TS, TS)] = jnp.where(
                    sub < 4, mid, ones)
                vt_scr[2 * j + 1, pl.ds(0, 8), pl.ds(r * TS, TS)] = jnp.where(
                    sub < 4, ones, mid)
                vt_scr[2 * j + 1, pl.ds(8, 16), pl.ds(r * TS, TS)] = (
                    vt[b + 24:b + 40])
        w, qtm = masked_qt(0, 0)
        mx = scores_chunk(w, qtm, 0)
        for c in range(1, S // TK):
            mx = jnp.maximum(mx, scores_chunk(w, qtm, c))
        finish_max(mx)

    def pair_step(j, carry):
        t_next = jnp.minimum(i * NPAIR + j + 1, NQ * NPAIR - 1)
        w, qtm = masked_qt(t_next // NPAIR, t_next % NPAIR)
        m8 = m_scr[...]
        acc_e = jnp.zeros((24, TQ), F32)
        acc_o = jnp.zeros((24, TQ), F32)
        mx = None
        for c in range(S // TK):
            s = s_scr[pl.ds(c * TK, TK), :].reshape(TK // 8, 8, 2 * TQ)
            p = jnp.exp2(s - m8[None]).reshape(TK, 2 * TQ).astype(BF16)
            acc_e = acc_e + jnp.dot(vt_scr[2 * j, :, pl.ds(c * TK, TK)],
                                    p[:, :TQ], preferred_element_type=F32)
            acc_o = acc_o + jnp.dot(vt_scr[2 * j + 1, :, pl.ds(c * TK, TK)],
                                    p[:, TQ:], preferred_element_type=F32)
            cm = scores_chunk(w, qtm, c)
            mx = cm if mx is None else jnp.maximum(mx, cm)
        finish_max(mx)
        o_e = acc_e / acc_e[20:21, :]
        o_o = acc_o / acc_o[0:1, :]
        sub = jax.lax.broadcasted_iota(jnp.int32, (8, TQ), 0)
        base = pl.multiple_of(40 * j, 8)
        ot_scr[pl.ds(base, 16), :] = o_e[0:16]
        ot_scr[pl.ds(base + 16, 8), :] = jnp.where(sub < 4, o_e[16:24], o_o[0:8])
        ot_scr[pl.ds(base + 24, 16), :] = o_o[8:24]
        return carry

    jax.lax.fori_loop(0, NPAIR, pair_step, 0)

    xs = x_ref[pl.ds(pl.multiple_of(i * TQ, TQ), TQ), :]
    a = jax.lax.dot_general(ot_scr[...].astype(BF16), wo_ref[...],
                            (((0,), (0,)), ((), ())),
                            preferred_element_type=F32)
    h = jnp.maximum(jnp.dot(xs, w1_ref[...], preferred_element_type=F32), 0.0)
    b = jnp.dot(h.astype(BF16), w2_ref[...], preferred_element_type=F32)
    z = jnp.sum(xs.astype(F32) * gw_ref[...].astype(F32), axis=-1, keepdims=True)
    g = jax.nn.sigmoid(z)
    o_ref[...] = (g * a + (1.0 - g) * b).astype(o_ref.dtype)


@jax.jit
def pallas_gated_mix__softmax_full_mha__dense_activation_relu__prompt_kernel(
    A_x: jax.Array,
    A_wqkv: jax.Array,
    A_wo: jax.Array,
    B_x: jax.Array,
    B_w1: jax.Array,
    B_w2: jax.Array,
    gate_w: jax.Array,
):
    del B_x
    x = A_x.reshape(S, D)
    gw = gate_w.reshape(1, D)
    full = lambda shape: pl.BlockSpec(shape, lambda i: (0,) * len(shape))
    out = pl.pallas_call(
        _kernel,
        grid=(NQ,),
        in_specs=[full((S, D)), full((D, 3 * D)), full((D, D)),
                  full((D, DFF)), full((DFF, D)), full((1, D))],
        out_specs=pl.BlockSpec((TQ, D), lambda i: (i, 0)),
        out_shape=jax.ShapeDtypeStruct((S, D), A_x.dtype),
        scratch_shapes=[
            pltpu.VMEM((NWIN, S, 128), BF16),
            pltpu.VMEM((NQ, NWIN, 128, TQ), BF16),
            pltpu.VMEM((H, 24, S), F32),
            pltpu.VMEM((S, 2 * TQ), F32),
            pltpu.VMEM((8, 2 * TQ), F32),
            pltpu.VMEM((D, TQ), F32),
        ],
        compiler_params=pltpu.CompilerParams(
            dimension_semantics=("arbitrary",),
            vmem_limit_bytes=100 * 1024 * 1024,
        ),
    )(x, A_wqkv, A_wo, B_w1, B_w2, gw)
    return out.reshape(A_x.shape)
```

```python
import math

import jax
import jax.numpy as jnp
import jax.experimental.pallas as pl
import jax.experimental.pallas.tpu as pltpu

S, D, H, DH, DFF = 2048, 640, 32, 20, 1536
NPAIR = H // 2
NWIN = 9
TQ = 256
NQ = S // TQ
TS = TQ
NR = S // TS
TK = 128
NC = S // TK
SKEW = 2
PEEL = 1
F32 = jnp.float32
BF16 = jnp.bfloat16
QSCALE = (DH ** -0.5) * math.log2(math.e)


def _kernel(x_hbm, wqkv_hbm, wo_hbm, w1_hbm, w2_hbm, gw_ref, o_ref,
            x_ref, wqkv_ref, wo_ref, w1_ref, w2_ref, sems,
            k_scr, qt_scr, vt_scr, s0_scr, s1_scr, m_scr, mx_scr, ot_scr):
    i = pl.program_id(0)
    s_bufs = (s0_scr, s1_scr)

    def x_copy(r):
        rows = pl.ds(r * TS, TS)
        return pltpu.make_async_copy(x_hbm.at[rows, :], x_ref.at[rows, :], sems.at[r])

    def wqkv_copy(part):
        return pltpu.make_async_copy(wqkv_hbm.at[:, pl.ds(part * D, D)],
                                     wqkv_ref.at[part], sems.at[NR + part])

    late_copies = (
        pltpu.make_async_copy(w1_hbm, w1_ref, sems.at[NR + 3]),
        pltpu.make_async_copy(w2_hbm, w2_ref, sems.at[NR + 4]),
        pltpu.make_async_copy(wo_hbm, wo_ref, sems.at[NR + 5]),
    )

    def masked_qt(qi, pj):
        w = min((40 * pj) // 64, NWIN - 1)
        qt = qt_scr[qi, w]
        row = jax.lax.broadcasted_iota(jnp.int32, (128, TQ), 0)
        rel = (row - 40 * pj) & 127
        zero = jnp.zeros_like(qt)
        qe = jnp.where(rel < DH, qt, zero)
        qo = jnp.where(jnp.logical_and(rel >= DH, rel < 2 * DH), qt, zero)
        return w, jnp.concatenate([qe, qo], axis=1)

    def scores_chunk(w, qtm, c, s_scr):
        s = jnp.dot(k_scr[w, pl.ds(c * TK, TK), :], qtm,
                    preferred_element_type=F32)
        s_scr[pl.ds(c * TK, TK), :] = s
        return jnp.max(s.reshape(TK // 8, 8, 2 * TQ), axis=0)

    def finish_max(mx):
        return jnp.broadcast_to(jnp.max(mx, axis=0, keepdims=True), (8, 2 * TQ))

    def row_slice(r):
        if isinstance(r, int):
            return pl.ds(r * TS, TS)
        return pl.ds(pl.multiple_of(r * TS, TS), TS)

    def proj_q(r):
        q = jnp.dot(x_ref[row_slice(r), :], wqkv_ref[0],
                    preferred_element_type=F32) * QSCALE
        qt = q.T.astype(BF16)
        for g in range(5):
            qt_scr[r, 2 * g] = qt[128 * g:128 * g + 128]
        for g in range(4):
            qt_scr[r, 2 * g + 1, pl.ds(0, 64), :] = qt[128 * (g + 1):128 * (g + 1) + 64]
            qt_scr[r, 2 * g + 1, pl.ds(64, 64), :] = qt[128 * g + 64:128 * g + 128]

    def proj_v(r):
        sub = jax.lax.broadcasted_iota(jnp.int32, (8, TS), 0)
        ones = jnp.ones((8, TS), F32)
        v = jnp.dot(x_ref[row_slice(r), :], wqkv_ref[2], preferred_element_type=F32)
        vt = v.astype(BF16).astype(F32).T
        for j in range(NPAIR):
            b = 40 * j
            mid = vt[b + 16:b + 24]
            vt_scr[r, 2 * j, pl.ds(0, 16), :] = vt[b:b + 16]
            vt_scr[r, 2 * j, pl.ds(16, 8), :] = jnp.where(sub < 4, mid, ones)
            vt_scr[r, 2 * j + 1, pl.ds(0, 8), :] = jnp.where(sub < 4, ones, mid)
            vt_scr[r, 2 * j + 1, pl.ds(8, 16), :] = vt[b + 24:b + 40]

    def proj_k(r):
        lane = jax.lax.broadcasted_iota(jnp.int32, (TS, 128), 1)
        rows = row_slice(r)
        k = jnp.dot(x_ref[rows, :], wqkv_ref[1], preferred_element_type=F32)
        for g in range(5):
            k_scr[2 * g, rows, :] = k[:, 128 * g:128 * g + 128].astype(BF16)
        for g in range(4):
            k_scr[2 * g + 1, rows, :] = jnp.where(
                lane >= 64, k[:, 128 * g:128 * g + 128],
                k[:, 128 * (g + 1):128 * (g + 1) + 128]).astype(BF16)

    @pl.when(i == 0)
    def _projections():
        x_copy(0).start()
        wqkv_copy(0).start()
        wqkv_copy(2).start()
        wqkv_copy(1).start()
        for r in range(1, NR):
            x_copy(r).start()
        if PEEL:
            x_copy(0).wait()
            wqkv_copy(0).wait()
            proj_q(0)
            wqkv_copy(2).wait()
            proj_v(0)
            wqkv_copy(1).wait()
            for cp in late_copies:
                cp.start()
            proj_k(0)
        else:
            for part in range(3):
                wqkv_copy(part).wait()
            for cp in late_copies:
                cp.start()

        def proj_chunk(r, carry):
            x_copy(r).wait()
            proj_q(r)
            proj_v(r)
            proj_k(r)
            return carry

        jax.lax.fori_loop(PEEL, NR, proj_chunk, 0)
        w, qtm = masked_qt(0, 0)
        mx = scores_chunk(w, qtm, 0, s0_scr)
        for c in range(1, NC):
            mx = jnp.maximum(mx, scores_chunk(w, qtm, c, s0_scr))
        m_scr[...] = finish_max(mx)
        w, qtm = masked_qt(0, 1)
        mx = scores_chunk(w, qtm, 0, s1_scr)
        for c in range(1, SKEW):
            mx = jnp.maximum(mx, scores_chunk(w, qtm, c, s1_scr))
        mx_scr[...] = mx
        for cp in late_copies:
            cp.wait()

    i_next = jnp.minimum(i + 1, NQ - 1)
    m_final = {0: m_scr[...]}
    mx = mx_scr[...]
    wq = masked_qt(i, 1)
    sub = jax.lax.broadcasted_iota(jnp.int32, (8, TQ), 0)
    for u in range(NPAIR * NC):
        j, c = divmod(u, NC)
        if c == 0:
            m_e = m_final[j][:, :TQ]
            m_o = m_final[j][:, TQ:]
            acc_e = jnp.zeros((24, TQ), F32)
            acc_o = jnp.zeros((24, TQ), F32)
        s_scr = s_bufs[j % 2]
        r, off = (c * TK) // TS, (c * TK) % TS
        s_e = s_scr[pl.ds(c * TK, TK), pl.ds(0, TQ)].reshape(TK // 8, 8, TQ)
        p_e = jnp.exp2(s_e - m_e[None]).reshape(TK, TQ).astype(BF16)
        acc_e = acc_e + jnp.dot(vt_scr[r, 2 * j, :, pl.ds(off, TK)],
                                p_e, preferred_element_type=F32)
        s_o = s_scr[pl.ds(c * TK, TK), pl.ds(TQ, TQ)].reshape(TK // 8, 8, TQ)
        p_o = jnp.exp2(s_o - m_o[None]).reshape(TK, TQ).astype(BF16)
        acc_o = acc_o + jnp.dot(vt_scr[r, 2 * j + 1, :, pl.ds(off, TK)],
                                p_o, preferred_element_type=F32)
        jn, cn = divmod(u + NC + SKEW, NC)
        if cn == 0:
            wq = masked_qt(i if jn < NPAIR else i_next, jn % NPAIR)
        cm = scores_chunk(wq[0], wq[1], cn, s_bufs[jn % 2])
        mx = cm if cn == 0 else jnp.maximum(mx, cm)
        if cn == NC - 1:
            m_final[jn] = finish_max(mx)
        if c == NC - 1:
            o_e = acc_e / acc_e[20:21, :]
            o_o = acc_o / acc_o[0:1, :]
            base = 40 * j
            ot_scr[pl.ds(base, 16), :] = o_e[0:16]
            ot_scr[pl.ds(base + 16, 8), :] = jnp.where(sub < 4, o_e[16:24], o_o[0:8])
            ot_scr[pl.ds(base + 24, 16), :] = o_o[8:24]
    m_scr[...] = m_final[NPAIR]
    mx_scr[...] = mx

    xs = x_ref[pl.ds(pl.multiple_of(i * TQ, TQ), TQ), :]
    h = jnp.maximum(jnp.dot(xs, w1_ref[...], preferred_element_type=F32), 0.0)
    b = jnp.dot(h.astype(BF16), w2_ref[...], preferred_element_type=F32)
    a = jax.lax.dot_general(ot_scr[...].astype(BF16), wo_ref[...],
                            (((0,), (0,)), ((), ())),
                            preferred_element_type=F32)
    z = jnp.sum(xs.astype(F32) * gw_ref[...].astype(F32), axis=-1, keepdims=True)
    g = jax.nn.sigmoid(z)
    o_ref[...] = (g * a + (1.0 - g) * b).astype(o_ref.dtype)


@jax.jit
def pallas_gated_mix__softmax_full_mha__dense_activation_relu__prompt_kernel(
    A_x: jax.Array,
    A_wqkv: jax.Array,
    A_wo: jax.Array,
    B_x: jax.Array,
    B_w1: jax.Array,
    B_w2: jax.Array,
    gate_w: jax.Array,
):
    del B_x
    x = A_x.reshape(S, D)
    gw = gate_w.reshape(1, D)
    full = lambda shape: pl.BlockSpec(shape, lambda i: (0,) * len(shape))
    out = pl.pallas_call(
        _kernel,
        grid=(NQ,),
        in_specs=[pl.BlockSpec(memory_space=pl.ANY)] * 5 + [full((1, D))],
        out_specs=pl.BlockSpec((TQ, D), lambda i: (i, 0)),
        out_shape=jax.ShapeDtypeStruct((S, D), A_x.dtype),
        scratch_shapes=[
            pltpu.VMEM((S, D), BF16),
            pltpu.VMEM((3, D, D), BF16),
            pltpu.VMEM((D, D), BF16),
            pltpu.VMEM((D, DFF), BF16),
            pltpu.VMEM((DFF, D), BF16),
            pltpu.SemaphoreType.DMA((NR + 6,)),
            pltpu.VMEM((NWIN, S, 128), BF16),
            pltpu.VMEM((NQ, NWIN, 128, TQ), BF16),
            pltpu.VMEM((NR, H, 24, TS), F32),
            pltpu.VMEM((S, 2 * TQ), F32),
            pltpu.VMEM((S, 2 * TQ), F32),
            pltpu.VMEM((8, 2 * TQ), F32),
            pltpu.VMEM((8, 2 * TQ), F32),
            pltpu.VMEM((D, TQ), F32),
        ],
        compiler_params=pltpu.CompilerParams(
            dimension_semantics=("arbitrary",),
            vmem_limit_bytes=100 * 1024 * 1024,
        ),
    )(x, A_wqkv, A_wo, B_w1, B_w2, gw)
    return out.reshape(A_x.shape)
```

```python
import math

import jax
import jax.numpy as jnp
import jax.experimental.pallas as pl
import jax.experimental.pallas.tpu as pltpu

S, D, H, DH, DFF = 2048, 640, 32, 20, 1536
NPAIR = H // 2
NWIN = 9
TQ = 256
NQ = S // TQ
TS = TQ
NR = S // TS
TK = 128
NC = S // TK
SKEW = 3
OFFC = 16
KG = OFFC // 8
NSUB = 5
F32 = jnp.float32
BF16 = jnp.bfloat16
U32 = jnp.uint32
QSCALE = (DH ** -0.5) * math.log2(math.e)


def _window(pj):
    return min((2 * DH * pj) // 64, NWIN - 1)


def _kernel(x_hbm, wqkv_hbm, wo_hbm, w1_hbm, w2_hbm, gw_hbm, o_ref,
            x_ref, wqkv_ref, wo_ref, w1_ref, w2_ref, sems,
            k_scr, kb_scr, qtf_scr, qb_scr, qh_scr, vt_scr, s0_scr, s1_scr,
            m_scr, mx_scr, ot_scr, ko_scr, gw_ref):
    i = pl.program_id(0)
    s_bufs = (s0_scr, s1_scr)

    def x_copy(r):
        rows = pl.ds(r * TS, TS)
        return pltpu.make_async_copy(x_hbm.at[rows, :], x_ref.at[rows, :], sems.at[r])

    def wqkv_copy(part):
        return pltpu.make_async_copy(wqkv_hbm.at[:, pl.ds(part * D, D)],
                                     wqkv_ref.at[part], sems.at[NR + part])

    late_copies = (
        pltpu.make_async_copy(w1_hbm, w1_ref, sems.at[NR + 3]),
        pltpu.make_async_copy(w2_hbm, w2_ref, sems.at[NR + 4]),
        pltpu.make_async_copy(wo_hbm, wo_ref, sems.at[NR + 5]),
        pltpu.make_async_copy(gw_hbm, gw_ref, sems.at[NR + 6]),
    )

    def q_weights(qi, pj):
        halves = []
        for hh in range(2):
            h = 2 * pj + hh
            t0 = ((DH * h) // 16) % 8
            blk = qh_scr[qi, h]
            tiles = [jnp.zeros((8, TQ), U32)] * 8
            tiles[t0] = blk[0:8]
            tiles[(t0 + 1) % 8] = blk[8:16]
            halves.append(jnp.concatenate(tiles, axis=0))
        return pltpu.bitcast(jnp.concatenate(halves, axis=1), BF16)

    def mxu_scores(qi, pj, c, s_scr):
        nrow = TK if c % 2 == 0 else TK - OFFC
        kc = pltpu.bitcast(
            k_scr[_window(pj), pl.ds(c * (TK // 2), nrow // 2), :], BF16)
        s = jnp.dot(kc, q_weights(qi, pj), preferred_element_type=F32)
        s_scr[pl.ds(c * TK, nrow), :] = s
        return jnp.max(s.reshape(nrow // 8, 8, 2 * TQ), axis=0)

    def vpu_piece(qi, pj, c, sub_i, accs):
        r, hh = divmod(c, 2)
        nd = DH // NSUB
        for d in range(sub_i * nd, (sub_i + 1) * nd):
            f = 2 * DH * pj + DH * hh + d
            if r == 0:
                qv = jnp.concatenate(
                    [jnp.broadcast_to(qtf_scr[qi, ct, pl.ds(f, 1), :], (8, 128))
                     for ct in range(TQ // 128)], axis=1)
                qb_scr[pj % 2, DH * hh + d] = qv
            else:
                qv = qb_scr[pj % 2, DH * hh + d]
            for kg in range(KG):
                kb = kb_scr[r, f, pl.ds(8 * kg, 8), :]
                t = jnp.concatenate([kb] * (TQ // 128), axis=1) * qv
                accs[kg] = t if accs[kg] is None else accs[kg] + t

    def vpu_finish(c, accs, s_scr, cm):
        r, hh = divmod(c, 2)
        neg = jnp.full((8, TQ), -jnp.inf, F32)
        for kg in range(KG):
            s_scr[pl.ds(r * TS + TS - OFFC + 8 * kg, 8), pl.ds(hh * TQ, TQ)] = accs[kg]
            cm = jnp.maximum(cm, jnp.concatenate(
                [accs[kg], neg] if hh == 0 else [neg, accs[kg]], axis=1))
        return cm

    def scores_chunk(qi, pj, c, s_scr):
        accs = [None] * KG
        for sub_i in range(NSUB):
            vpu_piece(qi, pj, c, sub_i, accs)
        return vpu_finish(c, accs, s_scr, mxu_scores(qi, pj, c, s_scr))

    def finish_max(mx):
        return jnp.broadcast_to(jnp.max(mx, axis=0, keepdims=True), (8, 2 * TQ))

    def row_slice(r, n):
        if isinstance(r, int):
            return pl.ds(r * n, n)
        return pl.ds(pl.multiple_of(r * n, n), n)

    def proj_q(r):
        q = jnp.dot(x_ref[row_slice(r, TS), :], wqkv_ref[0],
                    preferred_element_type=F32) * QSCALE
        qt = q.astype(BF16).astype(F32).T
        for ct in range(TQ // 128):
            qtf_scr[r, ct] = qt[:, 128 * ct:128 * (ct + 1)]
        row = jax.lax.broadcasted_iota(jnp.int32, (32, TQ), 0)
        for h in range(H):
            f0 = ((DH * h) // 16) * 16
            lo = DH * h - f0
            keep = jnp.logical_and(row >= lo, row < lo + DH)
            qh_scr[r, h] = pltpu.bitcast(
                jnp.where(keep, qt[f0:f0 + 32], 0.0).astype(BF16), U32)

    def proj_v(r):
        sub = jax.lax.broadcasted_iota(jnp.int32, (8, TS), 0)
        ones = jnp.ones((8, TS), F32)
        v = jnp.dot(x_ref[row_slice(r, TS), :], wqkv_ref[2], preferred_element_type=F32)
        vt = v.astype(BF16).astype(F32).T
        for j in range(NPAIR):
            b = 2 * DH * j
            mid = vt[b + 16:b + 24]
            vt_scr[r, 2 * j, pl.ds(0, 16), :] = vt[b:b + 16]
            vt_scr[r, 2 * j, pl.ds(16, 8), :] = jnp.where(sub < 4, mid, ones)
            vt_scr[r, 2 * j + 1, pl.ds(0, 8), :] = jnp.where(sub < 4, ones, mid)
            vt_scr[r, 2 * j + 1, pl.ds(8, 16), :] = vt[b + 24:b + 40]

    def proj_k(r):
        lane = jax.lax.broadcasted_iota(jnp.int32, (TS, 128), 1)
        hrows = row_slice(r, TS // 2)
        k = jnp.dot(x_ref[row_slice(r, TS), :], wqkv_ref[1], preferred_element_type=F32)
        k = k.astype(BF16).astype(F32)
        for g in range(5):
            k_scr[2 * g, hrows, :] = pltpu.bitcast(
                k[:, 128 * g:128 * g + 128].astype(BF16), U32)
        for g in range(4):
            k_scr[2 * g + 1, hrows, :] = pltpu.bitcast(jnp.where(
                lane >= 64, k[:, 128 * g:128 * g + 128],
                k[:, 128 * (g + 1):128 * (g + 1) + 128]).astype(BF16), U32)
        ko_scr[...] = k[TS - OFFC:, :].astype(BF16)

    def bcast_k(r):
        ko = ko_scr[...].astype(F32)
        for f in range(D):
            kb_scr[r, f] = jnp.broadcast_to(ko[:, f:f + 1], (OFFC, 128))

    @pl.when(i == 0)
    def _projections():
        x_copy(0).start()
        wqkv_copy(0).start()
        wqkv_copy(2).start()
        wqkv_copy(1).start()
        for r in range(1, NR):
            x_copy(r).start()
        x_copy(0).wait()
        wqkv_copy(0).wait()
        proj_q(0)
        wqkv_copy(2).wait()
        proj_v(0)
        wqkv_copy(1).wait()
        for cp in late_copies:
            cp.start()
        proj_k(0)

        def proj_chunk(r, carry):
            x_copy(r).wait()
            bcast_k(r - 1)
            proj_q(r)
            proj_v(r)
            proj_k(r)
            return carry

        jax.lax.fori_loop(1, NR, proj_chunk, 0)
        bcast_k(NR - 1)
        mx = scores_chunk(0, 0, 0, s0_scr)
        for c in range(1, NC):
            mx = jnp.maximum(mx, scores_chunk(0, 0, c, s0_scr))
        m_scr[...] = finish_max(mx)
        mx = scores_chunk(0, 1, 0, s1_scr)
        for c in range(1, SKEW):
            mx = jnp.maximum(mx, scores_chunk(0, 1, c, s1_scr))
        mx_scr[...] = mx
        for cp in late_copies:
            cp.wait()

    i_next = jnp.minimum(i + 1, NQ - 1)
    m_final = {0: m_scr[...]}
    mx = mx_scr[...]
    sub = jax.lax.broadcasted_iota(jnp.int32, (8, TQ), 0)
    for u in range(NPAIR * NC):
        j, c = divmod(u, NC)
        jn, cn = divmod(u + NC + SKEW, NC)
        qn = i if jn < NPAIR else i_next
        accs = [None] * KG
        pieces = list(range(NSUB))

        def piece():
            if pieces:
                vpu_piece(qn, jn % NPAIR, cn, pieces.pop(0), accs)

        if c == 0:
            m_e = m_final[j][:, :TQ]
            m_o = m_final[j][:, TQ:]
            acc_e = jnp.zeros((24, TQ), F32)
            acc_o = jnp.zeros((24, TQ), F32)
        s_scr = s_bufs[j % 2]
        r, off = divmod(c * TK, TS)
        s_e = s_scr[pl.ds(c * TK, TK), pl.ds(0, TQ)].reshape(TK // 8, 8, TQ)
        p_e = jnp.exp2(s_e - m_e[None]).reshape(TK, TQ).astype(BF16)
        piece()
        acc_e = acc_e + jnp.dot(vt_scr[r, 2 * j, :, pl.ds(off, TK)],
                                p_e, preferred_element_type=F32)
        piece()
        s_o = s_scr[pl.ds(c * TK, TK), pl.ds(TQ, TQ)].reshape(TK // 8, 8, TQ)
        p_o = jnp.exp2(s_o - m_o[None]).reshape(TK, TQ).astype(BF16)
        piece()
        acc_o = acc_o + jnp.dot(vt_scr[r, 2 * j + 1, :, pl.ds(off, TK)],
                                p_o, preferred_element_type=F32)
        piece()
        cm = mxu_scores(qn, jn % NPAIR, cn, s_bufs[jn % 2])
        while pieces:
            piece()
        cm = vpu_finish(cn, accs, s_bufs[jn % 2], cm)
        mx = cm if cn == 0 else jnp.maximum(mx, cm)
        if cn == NC - 1:
            m_final[jn] = finish_max(mx)
        if c == NC - 1:
            o_e = acc_e / acc_e[20:21, :]
            o_o = acc_o / acc_o[0:1, :]
            base = 2 * DH * j
            ot_scr[pl.ds(base, 16), :] = o_e[0:16]
            ot_scr[pl.ds(base + 16, 8), :] = jnp.where(sub < 4, o_e[16:24], o_o[0:8])
            ot_scr[pl.ds(base + 24, 16), :] = o_o[8:24]
    m_scr[...] = m_final[NPAIR]
    mx_scr[...] = mx

    xs = x_ref[pl.ds(pl.multiple_of(i * TQ, TQ), TQ), :]
    h = jnp.maximum(jnp.dot(xs, w1_ref[...], preferred_element_type=F32), 0.0)
    b = jnp.dot(h.astype(BF16), w2_ref[...], preferred_element_type=F32)
    a = jax.lax.dot_general(ot_scr[...].astype(BF16), wo_ref[...],
                            (((0,), (0,)), ((), ())),
                            preferred_element_type=F32)
    z = jnp.sum(xs.astype(F32) * gw_ref[...].astype(F32)[None, :],
                axis=-1, keepdims=True)
    g = jax.nn.sigmoid(z)
    o_ref[...] = (g * a + (1.0 - g) * b).astype(o_ref.dtype)


@jax.jit
def pallas_gated_mix__softmax_full_mha__dense_activation_relu__prompt_kernel(
    A_x: jax.Array,
    A_wqkv: jax.Array,
    A_wo: jax.Array,
    B_x: jax.Array,
    B_w1: jax.Array,
    B_w2: jax.Array,
    gate_w: jax.Array,
):
    del B_x
    out = pl.pallas_call(
        _kernel,
        grid=(NQ,),
        in_specs=[pl.BlockSpec(memory_space=pl.ANY)] * 6,
        out_specs=pl.BlockSpec((TQ, D), lambda i: (i, 0)),
        out_shape=jax.ShapeDtypeStruct((S, D), A_x.dtype),
        scratch_shapes=[
            pltpu.VMEM((S, D), BF16),
            pltpu.VMEM((3, D, D), BF16),
            pltpu.VMEM((D, D), BF16),
            pltpu.VMEM((D, DFF), BF16),
            pltpu.VMEM((DFF, D), BF16),
            pltpu.SemaphoreType.DMA((NR + 7,)),
            pltpu.VMEM((NWIN, S // 2, 128), U32),
            pltpu.VMEM((NR, D, OFFC, 128), F32),
            pltpu.VMEM((NQ, TQ // 128, D, 128), F32),
            pltpu.VMEM((2, 2 * DH, 8, TQ), F32),
            pltpu.VMEM((NQ, H, 16, TQ), U32),
            pltpu.VMEM((NR, H, 24, TS), F32),
            pltpu.VMEM((S, 2 * TQ), F32),
            pltpu.VMEM((S, 2 * TQ), F32),
            pltpu.VMEM((8, 2 * TQ), F32),
            pltpu.VMEM((8, 2 * TQ), F32),
            pltpu.VMEM((D, TQ), F32),
            pltpu.VMEM((OFFC, D), BF16),
            pltpu.VMEM((D,), BF16),
        ],
        compiler_params=pltpu.CompilerParams(
            dimension_semantics=("arbitrary",),
            vmem_limit_bytes=120 * 1024 * 1024,
        ),
    )(A_x.reshape(S, D), A_wqkv, A_wo, B_w1, B_w2, gate_w)
    return out.reshape(A_x.shape)
```

```python
import math

import jax
import jax.numpy as jnp
import jax.experimental.pallas as pl
import jax.experimental.pallas.tpu as pltpu

S, D, H, DH, DFF = 2048, 640, 32, 20, 1536
NPAIR = H // 2
NWIN = 9
TQ = 256
NQ = S // TQ
TS = TQ
NR = S // TS
TK = 128
NC = S // TK
SKEW = 3
OFFC = 16
KG = OFFC // 8
NSUB = 4
NPIN = 2
F32 = jnp.float32
BF16 = jnp.bfloat16
U32 = jnp.uint32
QSCALE = (DH ** -0.5) * math.log2(math.e)


def _window(pj):
    return min((2 * DH * pj) // 64, NWIN - 1)


def _kernel(x_hbm, wqkv_hbm, wo_hbm, w1_hbm, w2_hbm, gw_hbm, o_ref,
            x_ref, wqkv_ref, wo_ref, w1_ref, w2_ref, sems,
            k_scr, kb_scr, qtf_scr, qb_scr, qh_scr, vt_scr, s0_scr, s1_scr,
            m_scr, mx_scr, ot_scr, ko_scr, gw_ref):
    i = pl.program_id(0)
    s_bufs = (s0_scr, s1_scr)

    def x_copy(r):
        rows = pl.ds(r * TS, TS)
        return pltpu.make_async_copy(x_hbm.at[rows, :], x_ref.at[rows, :], sems.at[r])

    def wqkv_copy(part):
        return pltpu.make_async_copy(wqkv_hbm.at[:, pl.ds(part * D, D)],
                                     wqkv_ref.at[part], sems.at[NR + part])

    late_copies = (
        pltpu.make_async_copy(w1_hbm, w1_ref, sems.at[NR + 3]),
        pltpu.make_async_copy(w2_hbm, w2_ref, sems.at[NR + 4]),
        pltpu.make_async_copy(wo_hbm, wo_ref, sems.at[NR + 5]),
        pltpu.make_async_copy(gw_hbm, gw_ref, sems.at[NR + 6]),
    )

    def q_weights(qi, pj):
        halves = []
        for hh in range(2):
            h = 2 * pj + hh
            t0 = ((DH * h) // 16) % 8
            blk = qh_scr[qi, h]
            tiles = [jnp.zeros((8, TQ), U32)] * 8
            tiles[t0] = blk[0:8]
            tiles[(t0 + 1) % 8] = blk[8:16]
            halves.append(jnp.concatenate(tiles, axis=0))
        return pltpu.bitcast(jnp.concatenate(halves, axis=1), BF16)

    def mxu_scores(qi, pj, c, s_scr, halves=None):
        nrow = TK if c % 2 == 0 else TK - OFFC
        kc = pltpu.bitcast(
            k_scr[_window(pj), pl.ds(c * (TK // 2), nrow // 2), :], BF16)
        s = jnp.dot(kc, q_weights(qi, pj), preferred_element_type=F32)
        s_scr[pl.ds(c * TK, nrow), :] = s
        s3 = s.reshape(nrow // 8, 8, 2 * TQ)
        nparts = NPIN
        bounds = [(nrow // 8) * t // nparts for t in range(nparts + 1)]
        cm = None
        for t in range(nparts):
            pm = jnp.max(s3[bounds[t]:bounds[t + 1]], axis=0)
            cm = pm if cm is None else jnp.maximum(cm, pm)
            if halves is not None:
                halves.append(cm)
        return cm

    def vpu_piece(qi, pj, c, sub_i, accs):
        r, hh = divmod(c, 2)
        nd = DH // NSUB
        for d in range(sub_i * nd, (sub_i + 1) * nd):
            f = 2 * DH * pj + DH * hh + d
            if r == 0:
                qv = jnp.concatenate(
                    [jnp.broadcast_to(qtf_scr[qi, ct, pl.ds(f, 1), :], (8, 128))
                     for ct in range(TQ // 128)], axis=1)
                qb_scr[pj % 2, DH * hh + d] = qv
            else:
                qv = qb_scr[pj % 2, DH * hh + d]
            for kg in range(KG):
                kb = kb_scr[r, f, pl.ds(8 * kg, 8), :]
                t = jnp.concatenate([kb] * (TQ // 128), axis=1) * qv
                accs[kg] = t if accs[kg] is None else accs[kg] + t

    def vpu_finish(c, accs, s_scr, cm):
        r, hh = divmod(c, 2)
        neg = jnp.full((8, TQ), -jnp.inf, F32)
        for kg in range(KG):
            s_scr[pl.ds(r * TS + TS - OFFC + 8 * kg, 8), pl.ds(hh * TQ, TQ)] = accs[kg]
            cm = jnp.maximum(cm, jnp.concatenate(
                [accs[kg], neg] if hh == 0 else [neg, accs[kg]], axis=1))
        return cm

    def scores_chunk(qi, pj, c, s_scr):
        accs = [None] * KG
        for sub_i in range(NSUB):
            vpu_piece(qi, pj, c, sub_i, accs)
        return vpu_finish(c, accs, s_scr, mxu_scores(qi, pj, c, s_scr))

    def finish_max(mx):
        return jnp.broadcast_to(jnp.max(mx, axis=0, keepdims=True), (8, 2 * TQ))

    def row_slice(r, n):
        if isinstance(r, int):
            return pl.ds(r * n, n)
        return pl.ds(pl.multiple_of(r * n, n), n)

    def proj_q(r):
        q = jnp.dot(x_ref[row_slice(r, TS), :], wqkv_ref[0],
                    preferred_element_type=F32) * QSCALE
        qt = q.astype(BF16).astype(F32).T
        for ct in range(TQ // 128):
            qtf_scr[r, ct] = qt[:, 128 * ct:128 * (ct + 1)]
        row = jax.lax.broadcasted_iota(jnp.int32, (32, TQ), 0)
        for h in range(H):
            f0 = ((DH * h) // 16) * 16
            lo = DH * h - f0
            keep = jnp.logical_and(row >= lo, row < lo + DH)
            qh_scr[r, h] = pltpu.bitcast(
                jnp.where(keep, qt[f0:f0 + 32], 0.0).astype(BF16), U32)

    def proj_v(r):
        sub = jax.lax.broadcasted_iota(jnp.int32, (8, TS), 0)
        ones = jnp.ones((8, TS), F32)
        v = jnp.dot(x_ref[row_slice(r, TS), :], wqkv_ref[2], preferred_element_type=F32)
        vt = v.astype(BF16).astype(F32).T
        for j in range(NPAIR):
            b = 2 * DH * j
            mid = vt[b + 16:b + 24]
            vt_scr[r, 2 * j, pl.ds(0, 16), :] = vt[b:b + 16]
            vt_scr[r, 2 * j, pl.ds(16, 8), :] = jnp.where(sub < 4, mid, ones)
            vt_scr[r, 2 * j + 1, pl.ds(0, 8), :] = jnp.where(sub < 4, ones, mid)
            vt_scr[r, 2 * j + 1, pl.ds(8, 16), :] = vt[b + 24:b + 40]

    def proj_k(r):
        lane = jax.lax.broadcasted_iota(jnp.int32, (TS, 128), 1)
        hrows = row_slice(r, TS // 2)
        k = jnp.dot(x_ref[row_slice(r, TS), :], wqkv_ref[1], preferred_element_type=F32)
        k = k.astype(BF16).astype(F32)
        for g in range(5):
            k_scr[2 * g, hrows, :] = pltpu.bitcast(
                k[:, 128 * g:128 * g + 128].astype(BF16), U32)
        for g in range(4):
            k_scr[2 * g + 1, hrows, :] = pltpu.bitcast(jnp.where(
                lane >= 64, k[:, 128 * g:128 * g + 128],
                k[:, 128 * (g + 1):128 * (g + 1) + 128]).astype(BF16), U32)
        ko_scr[...] = k[TS - OFFC:, :].astype(BF16)

    def bcast_k(r):
        ko = ko_scr[...].astype(F32)
        for f in range(D):
            kb_scr[r, f] = jnp.broadcast_to(ko[:, f:f + 1], (OFFC, 128))

    @pl.when(i == 0)
    def _projections():
        x_copy(0).start()
        wqkv_copy(0).start()
        wqkv_copy(2).start()
        wqkv_copy(1).start()
        for r in range(1, NR):
            x_copy(r).start()
        x_copy(0).wait()
        wqkv_copy(0).wait()
        proj_q(0)
        wqkv_copy(2).wait()
        proj_v(0)
        wqkv_copy(1).wait()
        for cp in late_copies:
            cp.start()
        proj_k(0)

        def proj_chunk(r, carry):
            x_copy(r).wait()
            bcast_k(r - 1)
            proj_q(r)
            proj_v(r)
            proj_k(r)
            return carry

        jax.lax.fori_loop(1, NR, proj_chunk, 0)
        bcast_k(NR - 1)
        mx = scores_chunk(0, 0, 0, s0_scr)
        for c in range(1, NC):
            mx = jnp.maximum(mx, scores_chunk(0, 0, c, s0_scr))
        m_scr[...] = finish_max(mx)
        mx = scores_chunk(0, 1, 0, s1_scr)
        for c in range(1, SKEW):
            mx = jnp.maximum(mx, scores_chunk(0, 1, c, s1_scr))
        mx_scr[...] = mx
        for cp in late_copies:
            cp.wait()

    i_next = jnp.minimum(i + 1, NQ - 1)
    m_final = {0: m_scr[...]}
    mx = mx_scr[...]
    prev = mx
    sub = jax.lax.broadcasted_iota(jnp.int32, (8, TQ), 0)
    for u in range(NPAIR * NC):
        j, c = divmod(u, NC)
        jn, cn = divmod(u + NC + SKEW, NC)
        qn = i if jn < NPAIR else i_next

        if c == 0:
            m_e = m_final[j][:, :TQ]
            m_o = m_final[j][:, TQ:]
            acc_e = jnp.zeros((24, TQ), F32)
            acc_o = jnp.zeros((24, TQ), F32)
        s_scr = s_bufs[j % 2]
        r, off = divmod(c * TK, TS)
        s_e = s_scr[pl.ds(c * TK, TK), pl.ds(0, TQ)].reshape(TK // 8, 8, TQ)
        p_e = jnp.exp2(s_e - m_e[None]).reshape(TK, TQ).astype(BF16)
        acc_e = acc_e + jnp.dot(vt_scr[r, 2 * j, :, pl.ds(off, TK)],
                                p_e, preferred_element_type=F32)
        s_o = s_scr[pl.ds(c * TK, TK), pl.ds(TQ, TQ)].reshape(TK // 8, 8, TQ)
        p_o = jnp.exp2(s_o - m_o[None]).reshape(TK, TQ).astype(BF16)
        acc_o = acc_o + jnp.dot(vt_scr[r, 2 * j + 1, :, pl.ds(off, TK)],
                                p_o, preferred_element_type=F32)
        parts = []
        cm = mxu_scores(qn, jn % NPAIR, cn, s_bufs[jn % 2], parts)
        pins = [prev] + parts[:-1]
        prev = cm
        accs = None
        for t in range(NPIN):
            zv = jnp.where(pins[t][:, :TQ] > 0.0, 0.0, -0.0)
            acc_t = [zv] * KG
            for sub_i in range(t * NSUB // NPIN, (t + 1) * NSUB // NPIN):
                vpu_piece(qn, jn % NPAIR, cn, sub_i, acc_t)
            accs = acc_t if accs is None else [x + y for x, y in zip(accs, acc_t)]
        cm = vpu_finish(cn, accs, s_bufs[jn % 2], cm)
        mx = cm if cn == 0 else jnp.maximum(mx, cm)
        if cn == NC - 1:
            m_final[jn] = finish_max(mx)
        if c == NC - 1:
            o_e = acc_e / acc_e[20:21, :]
            o_o = acc_o / acc_o[0:1, :]
            base = 2 * DH * j
            ot_scr[pl.ds(base, 16), :] = o_e[0:16]
            ot_scr[pl.ds(base + 16, 8), :] = jnp.where(sub < 4, o_e[16:24], o_o[0:8])
            ot_scr[pl.ds(base + 24, 16), :] = o_o[8:24]
    m_scr[...] = m_final[NPAIR]
    mx_scr[...] = mx

    xs = x_ref[pl.ds(pl.multiple_of(i * TQ, TQ), TQ), :]
    h = jnp.maximum(jnp.dot(xs, w1_ref[...], preferred_element_type=F32), 0.0)
    b = jnp.dot(h.astype(BF16), w2_ref[...], preferred_element_type=F32)
    a = jax.lax.dot_general(ot_scr[...].astype(BF16), wo_ref[...],
                            (((0,), (0,)), ((), ())),
                            preferred_element_type=F32)
    z = jnp.sum(xs.astype(F32) * gw_ref[...].astype(F32)[None, :],
                axis=-1, keepdims=True)
    g = jax.nn.sigmoid(z)
    o_ref[...] = (g * a + (1.0 - g) * b).astype(o_ref.dtype)


@jax.jit
def pallas_gated_mix__softmax_full_mha__dense_activation_relu__prompt_kernel(
    A_x: jax.Array,
    A_wqkv: jax.Array,
    A_wo: jax.Array,
    B_x: jax.Array,
    B_w1: jax.Array,
    B_w2: jax.Array,
    gate_w: jax.Array,
):
    del B_x
    out = pl.pallas_call(
        _kernel,
        grid=(NQ,),
        in_specs=[pl.BlockSpec(memory_space=pl.ANY)] * 6,
        out_specs=pl.BlockSpec((TQ, D), lambda i: (i, 0)),
        out_shape=jax.ShapeDtypeStruct((S, D), A_x.dtype),
        scratch_shapes=[
            pltpu.VMEM((S, D), BF16),
            pltpu.VMEM((3, D, D), BF16),
            pltpu.VMEM((D, D), BF16),
            pltpu.VMEM((D, DFF), BF16),
            pltpu.VMEM((DFF, D), BF16),
            pltpu.SemaphoreType.DMA((NR + 7,)),
            pltpu.VMEM((NWIN, S // 2, 128), U32),
            pltpu.VMEM((NR, D, OFFC, 128), F32),
            pltpu.VMEM((NQ, TQ // 128, D, 128), F32),
            pltpu.VMEM((2, 2 * DH, 8, TQ), F32),
            pltpu.VMEM((NQ, H, 16, TQ), U32),
            pltpu.VMEM((NR, H, 24, TS), F32),
            pltpu.VMEM((S, 2 * TQ), F32),
            pltpu.VMEM((S, 2 * TQ), F32),
            pltpu.VMEM((8, 2 * TQ), F32),
            pltpu.VMEM((8, 2 * TQ), F32),
            pltpu.VMEM((D, TQ), F32),
            pltpu.VMEM((OFFC, D), BF16),
            pltpu.VMEM((D,), BF16),
        ],
        compiler_params=pltpu.CompilerParams(
            dimension_semantics=("arbitrary",),
            vmem_limit_bytes=120 * 1024 * 1024,
        ),
    )(A_x.reshape(S, D), A_wqkv, A_wo, B_w1, B_w2, gate_w)
    return out.reshape(A_x.shape)
```

```python
import math

import jax
import jax.numpy as jnp
import jax.experimental.pallas as pl
import jax.experimental.pallas.tpu as pltpu

S, D, H, DH, DFF = 2048, 640, 32, 20, 1536
NPAIR = H // 2
NWIN = 9
TQ = 256
NQ = S // TQ
TS = TQ
NR = S // TS
TK = 128
NC = S // TK
SKEW = 3
OFFC = 16
KG = OFFC // 8
NPIN = 2
F32 = jnp.float32
BF16 = jnp.bfloat16
U32 = jnp.uint32
QSCALE = (DH ** -0.5) * math.log2(math.e)


def _window(pj):
    return min((2 * DH * pj) // 64, NWIN - 1)


def _kernel(x_hbm, wqkv_hbm, wo_hbm, w1_hbm, w2_hbm, gw_hbm, o_ref,
            x_ref, wqkv_ref, wo_ref, w1_ref, w2_ref, sems,
            k_scr, kb_scr, qtf_scr, qb_scr, qh_scr, vt_scr, s0_scr, s1_scr,
            m_scr, mx_scr, ot_scr, ko_scr, gw_ref):
    i = pl.program_id(0)
    s_bufs = (s0_scr, s1_scr)

    def x_copy(r):
        rows = pl.ds(r * TS, TS)
        return pltpu.make_async_copy(x_hbm.at[rows, :], x_ref.at[rows, :], sems.at[r])

    def wqkv_copy(part):
        return pltpu.make_async_copy(wqkv_hbm.at[:, pl.ds(part * D, D)],
                                     wqkv_ref.at[part], sems.at[NR + part])

    late_copies = (
        pltpu.make_async_copy(w1_hbm, w1_ref, sems.at[NR + 3]),
        pltpu.make_async_copy(w2_hbm, w2_ref, sems.at[NR + 4]),
        pltpu.make_async_copy(wo_hbm, wo_ref, sems.at[NR + 5]),
        pltpu.make_async_copy(gw_hbm, gw_ref, sems.at[NR + 6]),
    )

    def q_weights(qi, pj):
        halves = []
        for hh in range(2):
            h = 2 * pj + hh
            t0 = ((DH * h) // 16) % 8
            blk = qh_scr[qi, h]
            tiles = [jnp.zeros((8, TQ), U32)] * 8
            tiles[t0] = blk[0:8]
            tiles[(t0 + 1) % 8] = blk[8:16]
            halves.append(jnp.concatenate(tiles, axis=0))
        return pltpu.bitcast(jnp.concatenate(halves, axis=1), BF16)

    def mxu_scores(qi, pj, c, s_scr, parts):
        nrow = TK if c % 2 == 0 else TK - OFFC
        kc = pltpu.bitcast(
            k_scr[_window(pj), pl.ds(c * (TK // 2), nrow // 2), :], BF16)
        s = jnp.dot(kc, q_weights(qi, pj), preferred_element_type=F32)
        s_scr[pl.ds(c * TK, nrow), :] = s
        s3 = s.reshape(nrow // 8, 8, 2 * TQ)
        bounds = [(nrow // 8) * t // NPIN for t in range(NPIN + 1)]
        cm = None
        for t in range(NPIN):
            pm = jnp.max(s3[bounds[t]:bounds[t + 1]], axis=0)
            cm = pm if cm is None else jnp.maximum(cm, pm)
            parts.append(cm)
        return cm

    def vpu_chain(qi, pj, c, t, init):
        r, hh = divmod(c, 2)
        nd = DH // NPIN
        d0 = DH * hh + t * nd
        f0 = 2 * DH * pj + d0
        if r == 0:
            qv = jnp.stack([jnp.concatenate(
                [jnp.broadcast_to(qtf_scr[qi, ct, pl.ds(f0 + d, 1), :], (8, 128))
                 for ct in range(TQ // 128)], axis=1) for d in range(nd)])
            qb_scr[pj % 2, pl.ds(d0, nd)] = qv
        else:
            qv = qb_scr[pj % 2, pl.ds(d0, nd)]
        kb = kb_scr[r, pl.ds(f0, nd)]
        kb = jnp.concatenate([kb] * (TQ // 128), axis=2).reshape(nd, KG, 8, TQ)
        terms = kb * qv[:, None]
        if init is not None:
            terms = jnp.concatenate(
                [jnp.broadcast_to(init[None, None], (1, KG, 8, TQ)), terms], axis=0)
        return jnp.sum(terms, axis=0)

    def vpu_finish(c, sv, s_scr, cm):
        r, hh = divmod(c, 2)
        s_scr[pl.ds(r * TS + TS - OFFC, OFFC), pl.ds(hh * TQ, TQ)] = sv.reshape(OFFC, TQ)
        neg = jnp.full((8, TQ), -jnp.inf, F32)
        vm = jnp.max(sv, axis=0)
        return jnp.maximum(cm, jnp.concatenate(
            [vm, neg] if hh == 0 else [neg, vm], axis=1))

    def scores_chunk(qi, pj, c, s_scr, prev):
        parts = []
        cm = mxu_scores(qi, pj, c, s_scr, parts)
        pins = [prev] + parts[:-1]
        sv = None
        for t in range(NPIN):
            zv = (None if pins[t] is None
                  else jnp.where(pins[t][:, :TQ] > 0.0, 0.0, -0.0))
            part = vpu_chain(qi, pj, c, t, zv)
            sv = part if sv is None else sv + part
        return vpu_finish(c, sv, s_scr, cm), cm

    def finish_max(mx):
        return jnp.broadcast_to(jnp.max(mx, axis=0, keepdims=True), (8, 2 * TQ))

    def row_slice(r, n):
        if isinstance(r, int):
            return pl.ds(r * n, n)
        return pl.ds(pl.multiple_of(r * n, n), n)

    def proj_q(r):
        q = jnp.dot(x_ref[row_slice(r, TS), :], wqkv_ref[0],
                    preferred_element_type=F32) * QSCALE
        qt = q.astype(BF16).astype(F32).T
        for ct in range(TQ // 128):
            qtf_scr[r, ct] = qt[:, 128 * ct:128 * (ct + 1)]
        row = jax.lax.broadcasted_iota(jnp.int32, (32, TQ), 0)
        for h in range(H):
            f0 = ((DH * h) // 16) * 16
            lo = DH * h - f0
            keep = jnp.logical_and(row >= lo, row < lo + DH)
            qh_scr[r, h] = pltpu.bitcast(
                jnp.where(keep, qt[f0:f0 + 32], 0.0).astype(BF16), U32)

    def proj_v(r):
        sub = jax.lax.broadcasted_iota(jnp.int32, (8, TS), 0)
        ones = jnp.ones((8, TS), F32)
        v = jnp.dot(x_ref[row_slice(r, TS), :], wqkv_ref[2], preferred_element_type=F32)
        vt = v.astype(BF16).astype(F32).T
        for j in range(NPAIR):
            b = 2 * DH * j
            mid = vt[b + 16:b + 24]
            vt_scr[r, 2 * j, pl.ds(0, 16), :] = vt[b:b + 16]
            vt_scr[r, 2 * j, pl.ds(16, 8), :] = jnp.where(sub < 4, mid, ones)
            vt_scr[r, 2 * j + 1, pl.ds(0, 8), :] = jnp.where(sub < 4, ones, mid)
            vt_scr[r, 2 * j + 1, pl.ds(8, 16), :] = vt[b + 24:b + 40]

    def proj_k(r):
        lane = jax.lax.broadcasted_iota(jnp.int32, (TS, 128), 1)
        hrows = row_slice(r, TS // 2)
        k = jnp.dot(x_ref[row_slice(r, TS), :], wqkv_ref[1], preferred_element_type=F32)
        k = k.astype(BF16).astype(F32)
        for g in range(5):
            k_scr[2 * g, hrows, :] = pltpu.bitcast(
                k[:, 128 * g:128 * g + 128].astype(BF16), U32)
        for g in range(4):
            k_scr[2 * g + 1, hrows, :] = pltpu.bitcast(jnp.where(
                lane >= 64, k[:, 128 * g:128 * g + 128],
                k[:, 128 * (g + 1):128 * (g + 1) + 128]).astype(BF16), U32)
        ko_scr[...] = k[TS - OFFC:, :].astype(BF16)

    def bcast_k(r):
        ko = ko_scr[...].astype(F32)
        for f in range(D):
            kb_scr[r, f] = jnp.broadcast_to(ko[:, f:f + 1], (OFFC, 128))

    @pl.when(i == 0)
    def _projections():
        x_copy(0).start()
        wqkv_copy(0).start()
        wqkv_copy(2).start()
        wqkv_copy(1).start()
        for r in range(1, NR):
            x_copy(r).start()
        x_copy(0).wait()
        wqkv_copy(0).wait()
        proj_q(0)
        wqkv_copy(2).wait()
        proj_v(0)
        wqkv_copy(1).wait()
        for cp in late_copies:
            cp.start()
        proj_k(0)

        def proj_chunk(r, carry):
            x_copy(r).wait()
            bcast_k(r - 1)
            proj_q(r)
            proj_v(r)
            proj_k(r)
            return carry

        jax.lax.fori_loop(1, NR, proj_chunk, 0)
        bcast_k(NR - 1)
        prev = None
        for v in range(NC + SKEW):
            jn, cn = divmod(v, NC)
            cm, prev = scores_chunk(0, jn, cn, s_bufs[jn], prev)
            mx = cm if cn == 0 else jnp.maximum(mx, cm)
            if cn == NC - 1:
                m_scr[...] = finish_max(mx)
        mx_scr[...] = mx
        for cp in late_copies:
            cp.wait()

    i_next = jnp.minimum(i + 1, NQ - 1)
    m_final = {0: m_scr[...]}
    mx = mx_scr[...]
    prev = mx
    sub = jax.lax.broadcasted_iota(jnp.int32, (8, TQ), 0)
    for u in range(NPAIR * NC):
        j, c = divmod(u, NC)
        jn, cn = divmod(u + NC + SKEW, NC)
        qn = i if jn < NPAIR else i_next
        if c == 0:
            m_e = m_final[j][:, :TQ]
            m_o = m_final[j][:, TQ:]
            acc_e = jnp.zeros((24, TQ), F32)
            acc_o = jnp.zeros((24, TQ), F32)
        s_scr = s_bufs[j % 2]
        r, off = divmod(c * TK, TS)
        s_e = s_scr[pl.ds(c * TK, TK), pl.ds(0, TQ)].reshape(TK // 8, 8, TQ)
        p_e = jnp.exp2(s_e - m_e[None]).reshape(TK, TQ).astype(BF16)
        acc_e = acc_e + jnp.dot(vt_scr[r, 2 * j, :, pl.ds(off, TK)],
                                p_e, preferred_element_type=F32)
        s_o = s_scr[pl.ds(c * TK, TK), pl.ds(TQ, TQ)].reshape(TK // 8, 8, TQ)
        p_o = jnp.exp2(s_o - m_o[None]).reshape(TK, TQ).astype(BF16)
        acc_o = acc_o + jnp.dot(vt_scr[r, 2 * j + 1, :, pl.ds(off, TK)],
                                p_o, preferred_element_type=F32)
        cm, prev = scores_chunk(qn, jn % NPAIR, cn, s_bufs[jn % 2], prev)
        mx = cm if cn == 0 else jnp.maximum(mx, cm)
        if cn == NC - 1:
            m_final[jn] = finish_max(mx)
        if c == NC - 1:
            o_e = acc_e / acc_e[20:21, :]
            o_o = acc_o / acc_o[0:1, :]
            base = 2 * DH * j
            ot_scr[pl.ds(base, 16), :] = o_e[0:16]
            ot_scr[pl.ds(base + 16, 8), :] = jnp.where(sub < 4, o_e[16:24], o_o[0:8])
            ot_scr[pl.ds(base + 24, 16), :] = o_o[8:24]
    m_scr[...] = m_final[NPAIR]
    mx_scr[...] = mx

    xs = x_ref[pl.ds(pl.multiple_of(i * TQ, TQ), TQ), :]
    h = jnp.maximum(jnp.dot(xs, w1_ref[...], preferred_element_type=F32), 0.0)
    b = jnp.dot(h.astype(BF16), w2_ref[...], preferred_element_type=F32)
    a = jax.lax.dot_general(ot_scr[...].astype(BF16), wo_ref[...],
                            (((0,), (0,)), ((), ())),
                            preferred_element_type=F32)
    z = jnp.sum(xs.astype(F32) * gw_ref[...].astype(F32)[None, :],
                axis=-1, keepdims=True)
    g = jax.nn.sigmoid(z)
    o_ref[...] = (g * a + (1.0 - g) * b).astype(o_ref.dtype)


@jax.jit
def pallas_gated_mix__softmax_full_mha__dense_activation_relu__prompt_kernel(
    A_x: jax.Array,
    A_wqkv: jax.Array,
    A_wo: jax.Array,
    B_x: jax.Array,
    B_w1: jax.Array,
    B_w2: jax.Array,
    gate_w: jax.Array,
):
    del B_x
    out = pl.pallas_call(
        _kernel,
        grid=(NQ,),
        in_specs=[pl.BlockSpec(memory_space=pl.ANY)] * 6,
        out_specs=pl.BlockSpec((TQ, D), lambda i: (i, 0)),
        out_shape=jax.ShapeDtypeStruct((S, D), A_x.dtype),
        scratch_shapes=[
            pltpu.VMEM((S, D), BF16),
            pltpu.VMEM((3, D, D), BF16),
            pltpu.VMEM((D, D), BF16),
            pltpu.VMEM((D, DFF), BF16),
            pltpu.VMEM((DFF, D), BF16),
            pltpu.SemaphoreType.DMA((NR + 7,)),
            pltpu.VMEM((NWIN, S // 2, 128), U32),
            pltpu.VMEM((NR, D, OFFC, 128), F32),
            pltpu.VMEM((NQ, TQ // 128, D, 128), F32),
            pltpu.VMEM((2, 2 * DH, 8, TQ), F32),
            pltpu.VMEM((NQ, H, 16, TQ), U32),
            pltpu.VMEM((NR, H, 24, TS), F32),
            pltpu.VMEM((S, 2 * TQ), F32),
            pltpu.VMEM((S, 2 * TQ), F32),
            pltpu.VMEM((8, 2 * TQ), F32),
            pltpu.VMEM((8, 2 * TQ), F32),
            pltpu.VMEM((D, TQ), F32),
            pltpu.VMEM((OFFC, D), BF16),
            pltpu.VMEM((D,), BF16),
        ],
        compiler_params=pltpu.CompilerParams(
            dimension_semantics=("arbitrary",),
            vmem_limit_bytes=120 * 1024 * 1024,
        ),
    )(A_x.reshape(S, D), A_wqkv, A_wo, B_w1, B_w2, gate_w)
    return out.reshape(A_x.shape)
```

```python
import math

import jax
import jax.numpy as jnp
import jax.experimental.pallas as pl
import jax.experimental.pallas.tpu as pltpu

S, D, H, DH, DFF = 2048, 640, 32, 20, 1536
NPAIR = H // 2
NWIN = 9
TQ = 256
NQ = S // TQ
TS = TQ
NR = S // TS
TK = 128
NC = S // TK
SKEW = 5
OFFC = 16
KG = OFFC // 8
NPIN = 2
F32 = jnp.float32
BF16 = jnp.bfloat16
U32 = jnp.uint32
QSCALE = (DH ** -0.5) * math.log2(math.e)


def _window(pj):
    return min((2 * DH * pj) // 64, NWIN - 1)


def _mxu_rows(c):
    if c < 2:
        return c * (TK - OFFC), TK - OFFC
    if c % 2 == 0 or c == NC - 1:
        return c * TK, TK
    return c * TK, TK - OFFC


def _vpu_row(r):
    return r * TS + TS - OFFC if r < NR - 1 else TS - 2 * OFFC


def _kernel(x_hbm, wqkv_hbm, wo_hbm, w1_hbm, w2_hbm, gw_hbm, o_ref,
            x_ref, wqkv_ref, wo_ref, w1_ref, w2_ref, sems,
            k_scr, kb_scr, qtf_scr, qb_scr, qh_scr, vt_scr, s0_scr, s1_scr,
            mx_scr, ot_scr, ko_scr, gw_ref):
    i = pl.program_id(0)
    s_bufs = (s0_scr, s1_scr)

    def x_copy(r):
        rows = pl.ds(r * TS, TS)
        return pltpu.make_async_copy(x_hbm.at[rows, :], x_ref.at[rows, :], sems.at[r])

    def wqkv_copy(part):
        return pltpu.make_async_copy(wqkv_hbm.at[:, pl.ds(part * D, D)],
                                     wqkv_ref.at[part], sems.at[NR + part])

    late_copies = (
        pltpu.make_async_copy(w1_hbm, w1_ref, sems.at[NR + 3]),
        pltpu.make_async_copy(w2_hbm, w2_ref, sems.at[NR + 4]),
        pltpu.make_async_copy(wo_hbm, wo_ref, sems.at[NR + 5]),
        pltpu.make_async_copy(gw_hbm, gw_ref, sems.at[NR + 6]),
    )

    def q_weights(qi, pj):
        halves = []
        for hh in range(2):
            h = 2 * pj + hh
            t0 = ((DH * h) // 16) % 8
            blk = qh_scr[qi, h]
            tiles = [jnp.zeros((8, TQ), U32)] * 8
            tiles[t0] = blk[0:8]
            tiles[(t0 + 1) % 8] = blk[8:16]
            halves.append(jnp.concatenate(tiles, axis=0))
        return pltpu.bitcast(jnp.concatenate(halves, axis=1), BF16)

    def mxu_scores(qi, pj, c, s_scr, parts):
        row0, nrow = _mxu_rows(c)
        kc = pltpu.bitcast(k_scr[_window(pj), pl.ds(row0 // 2, nrow // 2), :], BF16)
        s = jnp.dot(kc, q_weights(qi, pj), preferred_element_type=F32)
        s_scr[pl.ds(row0, nrow), :] = s
        s3 = s.reshape(nrow // 8, 8, 2 * TQ)
        bounds = [(nrow // 8) * t // NPIN for t in range(NPIN + 1)]
        cm = None
        for t in range(NPIN):
            pm = jnp.max(s3[bounds[t]:bounds[t + 1]], axis=0)
            cm = pm if cm is None else jnp.maximum(cm, pm)
            parts.append(cm)
        return cm

    def vpu_chain(qi, pj, c, t, init):
        r, hh = divmod(c, 2)
        nd = DH // NPIN
        d0 = DH * hh + t * nd
        f0 = 2 * DH * pj + d0
        if r == 0:
            qv = jnp.stack([jnp.concatenate(
                [jnp.broadcast_to(qtf_scr[qi, ct, pl.ds(f0 + d, 1), :], (8, 128))
                 for ct in range(TQ // 128)], axis=1) for d in range(nd)])
            qb_scr[pj % 2, pl.ds(d0, nd)] = qv
        else:
            qv = qb_scr[pj % 2, pl.ds(d0, nd)]
        kb = kb_scr[r, pl.ds(f0, nd)]
        kb = jnp.concatenate([kb] * (TQ // 128), axis=2).reshape(nd, KG, 8, TQ)
        terms = kb * qv[:, None]
        if init is not None:
            terms = jnp.concatenate(
                [jnp.broadcast_to(init[None, None], (1, KG, 8, TQ)), terms], axis=0)
        return jnp.sum(terms, axis=0)

    def vpu_finish(c, sv, s_scr, cm):
        r, hh = divmod(c, 2)
        s_scr[pl.ds(_vpu_row(r), OFFC), pl.ds(hh * TQ, TQ)] = sv.reshape(OFFC, TQ)
        neg = jnp.full((8, TQ), -jnp.inf, F32)
        vm = jnp.max(sv, axis=0)
        return jnp.maximum(cm, jnp.concatenate(
            [vm, neg] if hh == 0 else [neg, vm], axis=1))

    def scores_chunk(qi, pj, c, s_scr, prev):
        parts = []
        cm = mxu_scores(qi, pj, c, s_scr, parts)
        pins = [prev] + parts[:-1]
        sv = None
        for t in range(NPIN):
            zv = (None if pins[t] is None
                  else jnp.where(pins[t][:, :TQ] > 0.0, 0.0, -0.0))
            part = vpu_chain(qi, pj, c, t, zv)
            sv = part if sv is None else sv + part
        return vpu_finish(c, sv, s_scr, cm), cm

    def finish_max(mx):
        return jnp.broadcast_to(jnp.max(mx, axis=0, keepdims=True), (8, 2 * TQ))

    def row_slice(r, n):
        if isinstance(r, int):
            return pl.ds(r * n, n)
        return pl.ds(pl.multiple_of(r * n, n), n)

    def proj_q(r):
        q = jnp.dot(x_ref[row_slice(r, TS), :], wqkv_ref[0],
                    preferred_element_type=F32) * QSCALE
        qt = q.astype(BF16).astype(F32).T
        for ct in range(TQ // 128):
            qtf_scr[r, ct] = qt[:, 128 * ct:128 * (ct + 1)]
        row = jax.lax.broadcasted_iota(jnp.int32, (32, TQ), 0)
        for h in range(H):
            f0 = ((DH * h) // 16) * 16
            lo = DH * h - f0
            keep = jnp.logical_and(row >= lo, row < lo + DH)
            qh_scr[r, h] = pltpu.bitcast(
                jnp.where(keep, qt[f0:f0 + 32], 0.0).astype(BF16), U32)

    def proj_v(r):
        sub = jax.lax.broadcasted_iota(jnp.int32, (8, TS), 0)
        ones = jnp.ones((8, TS), F32)
        v = jnp.dot(x_ref[row_slice(r, TS), :], wqkv_ref[2], preferred_element_type=F32)
        vt = v.astype(BF16).astype(F32).T
        for j in range(NPAIR):
            b = 2 * DH * j
            mid = vt[b + 16:b + 24]
            vt_scr[r, 2 * j, pl.ds(0, 16), :] = vt[b:b + 16]
            vt_scr[r, 2 * j, pl.ds(16, 8), :] = jnp.where(sub < 4, mid, ones)
            vt_scr[r, 2 * j + 1, pl.ds(0, 8), :] = jnp.where(sub < 4, ones, mid)
            vt_scr[r, 2 * j + 1, pl.ds(8, 16), :] = vt[b + 24:b + 40]

    def proj_k(r):
        lane = jax.lax.broadcasted_iota(jnp.int32, (TS, 128), 1)
        hrows = row_slice(r, TS // 2)
        k = jnp.dot(x_ref[row_slice(r, TS), :], wqkv_ref[1], preferred_element_type=F32)
        k = k.astype(BF16).astype(F32)
        for g in range(5):
            k_scr[2 * g, hrows, :] = pltpu.bitcast(
                k[:, 128 * g:128 * g + 128].astype(BF16), U32)
        for g in range(4):
            k_scr[2 * g + 1, hrows, :] = pltpu.bitcast(jnp.where(
                lane >= 64, k[:, 128 * g:128 * g + 128],
                k[:, 128 * (g + 1):128 * (g + 1) + 128]).astype(BF16), U32)
        ko_scr[...] = k[TS - 2 * OFFC:, :].astype(BF16)

    def bcast_k(r, half, f_lo=0, f_hi=D):
        ko = ko_scr[pl.ds(half * OFFC, OFFC), :].astype(F32)
        for f in range(f_lo, f_hi):
            kb_scr[r, f] = jnp.broadcast_to(ko[:, f:f + 1], (OFFC, 128))

    def lookahead(qi, jn):
        cm, _ = scores_chunk(qi, jn, 0, s_bufs[jn], None)
        mx_scr[jn] = cm

    @pl.when(i == 0)
    def _projections():
        x_copy(0).start()
        wqkv_copy(1).start()
        wqkv_copy(0).start()
        wqkv_copy(2).start()
        for r in range(1, NR):
            x_copy(r).start()
        x_copy(0).wait()
        wqkv_copy(1).wait()
        proj_k(0)
        wqkv_copy(0).wait()
        bcast_k(NR - 1, 0, 0, D // 2)
        proj_q(0)
        wqkv_copy(2).wait()
        for cp in late_copies:
            cp.start()
        bcast_k(NR - 1, 0, D // 2, D)
        proj_v(0)

        def proj_chunk(r, carry):
            x_copy(r).wait()
            bcast_k(r - 1, 1)
            proj_q(r)
            proj_v(r)
            proj_k(r)
            return carry

        jax.lax.fori_loop(1, NR, proj_chunk, 0)
        lookahead(0, 0)
        lookahead(0, 1)
        for cp in late_copies:
            cp.wait()

    i_next = jnp.minimum(i + 1, NQ - 1)
    xs = x_ref[pl.ds(pl.multiple_of(i * TQ, TQ), TQ), :]
    sub = jax.lax.broadcasted_iota(jnp.int32, (8, TQ), 0)
    todo = [(jn, cn) for jn in range(NPAIR) for cn in range(NC) if jn > 1 or cn > 0]
    m_final = {}
    st = {"prev": None, "mx": None}

    def produce():
        jn, cn = todo.pop(0)
        cm, st["prev"] = scores_chunk(i, jn, cn, s_bufs[jn % 2], st["prev"])
        if jn <= 1 and cn == 1:
            st["mx"] = mx_scr[jn]
        st["mx"] = cm if cn == 0 else jnp.maximum(st["mx"], cm)
        if cn == NC - 1:
            m_final[jn] = finish_max(st["mx"])

    ffn_units = [(nb, rh, kt) for nb in range(DFF // 512) for rh in range(2)
                 for kt in range(D // 128)]
    hacc = {}

    def ffn_unit():
        nb, rh, kt = ffn_units.pop(0)
        part = jnp.dot(xs[128 * rh:128 * (rh + 1), 128 * kt:128 * (kt + 1)],
                       w1_ref[pl.ds(128 * kt, 128), pl.ds(512 * nb, 512)],
                       preferred_element_type=F32)
        hacc[nb, rh] = part if kt == 0 else hacc[nb, rh] + part

    for _ in range(NC + SKEW - 2):
        produce()
    for u in range(NPAIR * NC):
        j, c = divmod(u, NC)
        if c == 0:
            m_e = m_final[j][:, :TQ]
            m_o = m_final[j][:, TQ:]
            acc_e = jnp.zeros((24, TQ), F32)
            acc_o = jnp.zeros((24, TQ), F32)
        s_scr = s_bufs[j % 2]
        r, off = divmod(c * TK, TS)
        s_e = s_scr[pl.ds(c * TK, TK), pl.ds(0, TQ)].reshape(TK // 8, 8, TQ)
        p_e = jnp.exp2(s_e - m_e[None]).reshape(TK, TQ).astype(BF16)
        acc_e = acc_e + jnp.dot(vt_scr[r, 2 * j, :, pl.ds(off, TK)],
                                p_e, preferred_element_type=F32)
        s_o = s_scr[pl.ds(c * TK, TK), pl.ds(TQ, TQ)].reshape(TK // 8, 8, TQ)
        p_o = jnp.exp2(s_o - m_o[None]).reshape(TK, TQ).astype(BF16)
        acc_o = acc_o + jnp.dot(vt_scr[r, 2 * j + 1, :, pl.ds(off, TK)],
                                p_o, preferred_element_type=F32)
        if todo:
            produce()
        elif u == NPAIR * NC - 8:
            lookahead(i_next, 0)
        elif u == NPAIR * NC - 4:
            lookahead(i_next, 1)
        else:
            ffn_unit()
        if c == NC - 1:
            o_e = acc_e / acc_e[20:21, :]
            o_o = acc_o / acc_o[0:1, :]
            base = 2 * DH * j
            ot_scr[pl.ds(base, 16), :] = o_e[0:16]
            ot_scr[pl.ds(base + 16, 8), :] = jnp.where(sub < 4, o_e[16:24], o_o[0:8])
            ot_scr[pl.ds(base + 24, 16), :] = o_o[8:24]

    while ffn_units:
        ffn_unit()
    h = jnp.concatenate(
        [jnp.concatenate([hacc[nb, rh] for nb in range(DFF // 512)], axis=1)
         for rh in range(2)], axis=0)
    b = jnp.dot(jnp.maximum(h, 0.0).astype(BF16), w2_ref[...],
                preferred_element_type=F32)
    a = jax.lax.dot_general(ot_scr[...].astype(BF16), wo_ref[...],
                            (((0,), (0,)), ((), ())),
                            preferred_element_type=F32)
    z = jnp.sum(xs.astype(F32) * gw_ref[...].astype(F32)[None, :],
                axis=-1, keepdims=True)
    g = jax.nn.sigmoid(z)
    o_ref[...] = (g * a + (1.0 - g) * b).astype(o_ref.dtype)


@jax.jit
def pallas_gated_mix__softmax_full_mha__dense_activation_relu__prompt_kernel(
    A_x: jax.Array,
    A_wqkv: jax.Array,
    A_wo: jax.Array,
    B_x: jax.Array,
    B_w1: jax.Array,
    B_w2: jax.Array,
    gate_w: jax.Array,
):
    del B_x
    out = pl.pallas_call(
        _kernel,
        grid=(NQ,),
        in_specs=[pl.BlockSpec(memory_space=pl.ANY)] * 6,
        out_specs=pl.BlockSpec((TQ, D), lambda i: (i, 0)),
        out_shape=jax.ShapeDtypeStruct((S, D), A_x.dtype),
        scratch_shapes=[
            pltpu.VMEM((S, D), BF16),
            pltpu.VMEM((3, D, D), BF16),
            pltpu.VMEM((D, D), BF16),
            pltpu.VMEM((D, DFF), BF16),
            pltpu.VMEM((DFF, D), BF16),
            pltpu.SemaphoreType.DMA((NR + 7,)),
            pltpu.VMEM((NWIN, S // 2, 128), U32),
            pltpu.VMEM((NR, D, OFFC, 128), F32),
            pltpu.VMEM((NQ, TQ // 128, D, 128), F32),
            pltpu.VMEM((2, 2 * DH, 8, TQ), F32),
            pltpu.VMEM((NQ, H, 16, TQ), U32),
            pltpu.VMEM((NR, H, 24, TS), F32),
            pltpu.VMEM((S, 2 * TQ), F32),
            pltpu.VMEM((S, 2 * TQ), F32),
            pltpu.VMEM((2, 8, 2 * TQ), F32),
            pltpu.VMEM((D, TQ), F32),
            pltpu.VMEM((2 * OFFC, D), BF16),
            pltpu.VMEM((D,), BF16),
        ],
        compiler_params=pltpu.CompilerParams(
            dimension_semantics=("arbitrary",),
            vmem_limit_bytes=120 * 1024 * 1024,
        ),
    )(A_x.reshape(S, D), A_wqkv, A_wo, B_w1, B_w2, gate_w)
    return out.reshape(A_x.shape)
```

```python
import math

import jax
import jax.numpy as jnp
import jax.experimental.pallas as pl
import jax.experimental.pallas.tpu as pltpu

S, D, H, DH, DFF = 2048, 640, 32, 20, 1536
NPAIR = H // 2
NWIN = 9
TQ = 256
NQ = S // TQ
TS = TQ
NR = S // TS
TK = 128
NC = S // TK
SKEW = 5
OFFC = 16
KG = OFFC // 8
NPIN = 2
F32 = jnp.float32
BF16 = jnp.bfloat16
U32 = jnp.uint32
QSCALE = (DH ** -0.5) * math.log2(math.e)


def _window(pj):
    return min((2 * DH * pj) // 64, NWIN - 1)


def _mxu_rows(c):
    if c < 2:
        return c * (TK - OFFC), TK - OFFC
    if c % 2 == 0 or c == NC - 1:
        return c * TK, TK
    return c * TK, TK - OFFC


def _vpu_row(r):
    return r * TS + TS - OFFC if r < NR - 1 else TS - 2 * OFFC


def _kernel(x_hbm, wqkv_hbm, wo_hbm, w1_hbm, w2_hbm, gw_hbm, o_ref,
            x_ref, wqkv_ref, wo_ref, w1_ref, w2_ref, sems,
            k_scr, kb_scr, qtf_scr, qb_scr, qh_scr, vt_scr, s0_scr, s1_scr,
            mx_scr, ot_scr, ko_scr, gw_ref):
    i = pl.program_id(0)
    s_bufs = (s0_scr, s1_scr)

    def x_copy(r):
        rows = pl.ds(r * TS, TS)
        return pltpu.make_async_copy(x_hbm.at[rows, :], x_ref.at[rows, :], sems.at[r])

    def wqkv_copy(part):
        return pltpu.make_async_copy(wqkv_hbm.at[:, pl.ds(part * D, D)],
                                     wqkv_ref.at[part], sems.at[NR + part])

    late_copies = (
        pltpu.make_async_copy(w1_hbm, w1_ref, sems.at[NR + 3]),
        pltpu.make_async_copy(w2_hbm, w2_ref, sems.at[NR + 4]),
        pltpu.make_async_copy(wo_hbm, wo_ref, sems.at[NR + 5]),
        pltpu.make_async_copy(gw_hbm, gw_ref, sems.at[NR + 6]),
    )

    def q_weights(qi, pj):
        halves = []
        for hh in range(2):
            h = 2 * pj + hh
            t0 = ((DH * h) // 16) % 8
            blk = qh_scr[qi, h]
            tiles = [jnp.zeros((8, TQ), U32)] * 8
            tiles[t0] = blk[0:8]
            tiles[(t0 + 1) % 8] = blk[8:16]
            halves.append(jnp.concatenate(tiles, axis=0))
        return pltpu.bitcast(jnp.concatenate(halves, axis=1), BF16)

    def mxu_scores(qi, pj, c, s_scr, parts):
        row0, nrow = _mxu_rows(c)
        kc = pltpu.bitcast(k_scr[_window(pj), pl.ds(row0 // 2, nrow // 2), :], BF16)
        s = jnp.dot(kc, q_weights(qi, pj), preferred_element_type=F32)
        s_scr[pl.ds(row0, nrow), :] = s
        s3 = s.reshape(nrow // 8, 8, 2 * TQ)
        bounds = [(nrow // 8) * t // NPIN for t in range(NPIN + 1)]
        cm = None
        for t in range(NPIN):
            pm = jnp.max(s3[bounds[t]:bounds[t + 1]], axis=0)
            cm = pm if cm is None else jnp.maximum(cm, pm)
            parts.append(cm)
        return cm

    def vpu_chain(qi, pj, c, t, init):
        r, hh = divmod(c, 2)
        nd = DH // NPIN
        d0 = DH * hh + t * nd
        f0 = 2 * DH * pj + d0
        qv = qb_scr[pl.ds(f0, nd)]
        kb = kb_scr[r, pl.ds(f0, nd)]
        kb = jnp.concatenate([kb] * (TQ // 128), axis=2).reshape(nd, KG, 8, TQ)
        terms = kb * qv[:, None]
        if init is not None:
            terms = jnp.concatenate(
                [jnp.broadcast_to(init[None, None], (1, KG, 8, TQ)), terms], axis=0)
        return jnp.sum(terms, axis=0)

    def stage_q(qi, f0, n, zv=None):
        for d in range(n):
            row = jnp.concatenate(
                [jnp.broadcast_to(qtf_scr[qi, ct, pl.ds(f0 + d, 1), :], (8, 128))
                 for ct in range(TQ // 128)], axis=1)
            qb_scr[f0 + d] = row if zv is None else row + zv

    def vpu_finish(c, sv, s_scr, cm):
        r, hh = divmod(c, 2)
        s_scr[pl.ds(_vpu_row(r), OFFC), pl.ds(hh * TQ, TQ)] = sv.reshape(OFFC, TQ)
        neg = jnp.full((8, TQ), -jnp.inf, F32)
        vm = jnp.max(sv, axis=0)
        return jnp.maximum(cm, jnp.concatenate(
            [vm, neg] if hh == 0 else [neg, vm], axis=1))

    def scores_chunk(qi, pj, c, s_scr, prev):
        parts = []
        cm = mxu_scores(qi, pj, c, s_scr, parts)
        pins = [prev] + parts[:-1]
        sv = None
        for t in range(NPIN):
            zv = (None if pins[t] is None
                  else jnp.where(pins[t][:, :TQ] > 0.0, 0.0, -0.0))
            part = vpu_chain(qi, pj, c, t, zv)
            sv = part if sv is None else sv + part
        return vpu_finish(c, sv, s_scr, cm), cm

    def finish_max(mx):
        return jnp.broadcast_to(jnp.max(mx, axis=0, keepdims=True), (8, 2 * TQ))

    def row_slice(r, n):
        if isinstance(r, int):
            return pl.ds(r * n, n)
        return pl.ds(pl.multiple_of(r * n, n), n)

    def proj_q(r):
        q = jnp.dot(x_ref[row_slice(r, TS), :], wqkv_ref[0],
                    preferred_element_type=F32) * QSCALE
        qt = q.astype(BF16).astype(F32).T
        for ct in range(TQ // 128):
            qtf_scr[r, ct] = qt[:, 128 * ct:128 * (ct + 1)]
        row = jax.lax.broadcasted_iota(jnp.int32, (32, TQ), 0)
        for h in range(H):
            f0 = ((DH * h) // 16) * 16
            lo = DH * h - f0
            keep = jnp.logical_and(row >= lo, row < lo + DH)
            qh_scr[r, h] = pltpu.bitcast(
                jnp.where(keep, qt[f0:f0 + 32], 0.0).astype(BF16), U32)

    def proj_v(r):
        sub = jax.lax.broadcasted_iota(jnp.int32, (8, TS), 0)
        ones = jnp.ones((8, TS), F32)
        v = jnp.dot(x_ref[row_slice(r, TS), :], wqkv_ref[2], preferred_element_type=F32)
        vt = v.astype(BF16).astype(F32).T
        for j in range(NPAIR):
            b = 2 * DH * j
            mid = vt[b + 16:b + 24]
            vt_scr[r, 2 * j, pl.ds(0, 16), :] = vt[b:b + 16]
            vt_scr[r, 2 * j, pl.ds(16, 8), :] = jnp.where(sub < 4, mid, ones)
            vt_scr[r, 2 * j + 1, pl.ds(0, 8), :] = jnp.where(sub < 4, ones, mid)
            vt_scr[r, 2 * j + 1, pl.ds(8, 16), :] = vt[b + 24:b + 40]

    def proj_k(r):
        lane = jax.lax.broadcasted_iota(jnp.int32, (TS, 128), 1)
        hrows = row_slice(r, TS // 2)
        k = jnp.dot(x_ref[row_slice(r, TS), :], wqkv_ref[1], preferred_element_type=F32)
        k = k.astype(BF16).astype(F32)
        for g in range(5):
            k_scr[2 * g, hrows, :] = pltpu.bitcast(
                k[:, 128 * g:128 * g + 128].astype(BF16), U32)
        for g in range(4):
            k_scr[2 * g + 1, hrows, :] = pltpu.bitcast(jnp.where(
                lane >= 64, k[:, 128 * g:128 * g + 128],
                k[:, 128 * (g + 1):128 * (g + 1) + 128]).astype(BF16), U32)
        ko_scr[...] = k[TS - 2 * OFFC:, :].astype(BF16)

    def bcast_k(r, half, f_lo=0, f_hi=D):
        ko = ko_scr[pl.ds(half * OFFC, OFFC), :].astype(F32)
        for f in range(f_lo, f_hi):
            kb_scr[r, f] = jnp.broadcast_to(ko[:, f:f + 1], (OFFC, 128))

    def lookahead(qi, jn):
        cm, _ = scores_chunk(qi, jn, 0, s_bufs[jn], None)
        mx_scr[jn] = cm

    @pl.when(i == 0)
    def _projections():
        x_copy(0).start()
        wqkv_copy(1).start()
        wqkv_copy(0).start()
        wqkv_copy(2).start()
        for r in range(1, NR):
            x_copy(r).start()
        x_copy(0).wait()
        wqkv_copy(1).wait()
        proj_k(0)
        wqkv_copy(0).wait()
        bcast_k(NR - 1, 0, 0, D // 2)
        proj_q(0)
        wqkv_copy(2).wait()
        for cp in late_copies:
            cp.start()
        bcast_k(NR - 1, 0, D // 2, D)
        proj_v(0)

        def proj_chunk(r, carry):
            x_copy(r).wait()
            bcast_k(r - 1, 1)
            stage_q(0, jnp.minimum((r - 1) * 92, D - 92), 92)
            proj_q(r)
            proj_v(r)
            proj_k(r)
            return carry

        jax.lax.fori_loop(1, NR, proj_chunk, 0)
        lookahead(0, 0)
        lookahead(0, 1)
        for cp in late_copies:
            cp.wait()

    i_next = jnp.minimum(i + 1, NQ - 1)
    xs = x_ref[pl.ds(pl.multiple_of(i * TQ, TQ), TQ), :]
    sub = jax.lax.broadcasted_iota(jnp.int32, (8, TQ), 0)
    todo = [(jn, cn) for jn in range(NPAIR) for cn in range(NC) if jn > 1 or cn > 0]
    m_final = {}
    st = {"prev": None, "mx": None, "staged": 0}

    def produce():
        jn, cn = todo.pop(0)
        cm, st["prev"] = scores_chunk(i, jn, cn, s_bufs[jn % 2], st["prev"])
        if jn <= 1 and cn == 1:
            st["mx"] = mx_scr[jn]
        st["mx"] = cm if cn == 0 else jnp.maximum(st["mx"], cm)
        if cn == NC - 1:
            m_final[jn] = finish_max(st["mx"])

    ffn_units = [(nb, rh, kt) for nb in range(DFF // 512) for rh in range(2)
                 for kt in range(D // 128)]
    hacc = {}

    def stage_next(src, n):
        n = min(n, D - st["staged"])
        if n > 0:
            stage_q(i_next, st["staged"], n, jnp.where(src > 0.0, 0.0, -0.0))
            st["staged"] += n

    def ffn_unit(nstage):
        nb, rh, kt = ffn_units.pop(0)
        part = jnp.dot(xs[128 * rh:128 * (rh + 1), 128 * kt:128 * (kt + 1)],
                       w1_ref[pl.ds(128 * kt, 128), pl.ds(512 * nb, 512)],
                       preferred_element_type=F32)
        hacc[nb, rh] = part if kt == 0 else hacc[nb, rh] + part
        stage_next(part[0:8, 0:TQ], nstage // 2)
        stage_next(part[64:72, 0:TQ], nstage // 2)

    for _ in range(NC + SKEW - 2):
        produce()
    for u in range(NPAIR * NC):
        j, c = divmod(u, NC)
        if c == 0:
            m_e = m_final[j][:, :TQ]
            m_o = m_final[j][:, TQ:]
            acc_e = jnp.zeros((24, TQ), F32)
            acc_o = jnp.zeros((24, TQ), F32)
        s_scr = s_bufs[j % 2]
        r, off = divmod(c * TK, TS)
        s_e = s_scr[pl.ds(c * TK, TK), pl.ds(0, TQ)].reshape(TK // 8, 8, TQ)
        p_e = jnp.exp2(s_e - m_e[None]).reshape(TK, TQ).astype(BF16)
        acc_e = acc_e + jnp.dot(vt_scr[r, 2 * j, :, pl.ds(off, TK)],
                                p_e, preferred_element_type=F32)
        s_o = s_scr[pl.ds(c * TK, TK), pl.ds(TQ, TQ)].reshape(TK // 8, 8, TQ)
        p_o = jnp.exp2(s_o - m_o[None]).reshape(TK, TQ).astype(BF16)
        acc_o = acc_o + jnp.dot(vt_scr[r, 2 * j + 1, :, pl.ds(off, TK)],
                                p_o, preferred_element_type=F32)
        if todo:
            produce()
        elif u == NPAIR * NC - 8:
            lookahead(i_next, 0)
        elif u == NPAIR * NC - 4:
            lookahead(i_next, 1)
        else:
            ffn_unit(10 if st["staged"] < 4 * DH else 0)
        if c == NC - 1:
            o_e = acc_e / acc_e[20:21, :]
            o_o = acc_o / acc_o[0:1, :]
            base = 2 * DH * j
            ot_scr[pl.ds(base, 16), :] = o_e[0:16]
            ot_scr[pl.ds(base + 16, 8), :] = jnp.where(sub < 4, o_e[16:24], o_o[0:8])
            ot_scr[pl.ds(base + 24, 16), :] = o_o[8:24]

    while ffn_units:
        ffn_unit(16)
    hs = [jnp.maximum(jnp.concatenate([hacc[nb, 0], hacc[nb, 1]], axis=0), 0.0).astype(BF16)
          for nb in range(DFF // 512)]
    bs = []
    for nt in range(D // 128):
        bacc = None
        for nb in range(DFF // 512):
            part = jnp.dot(hs[nb], w2_ref[pl.ds(512 * nb, 512), pl.ds(128 * nt, 128)],
                           preferred_element_type=F32)
            for t in range(4):
                stage_next(jnp.concatenate(
                    [part[64 * t:64 * t + 8], part[64 * t + 8:64 * t + 16]], axis=1), 7)
            bacc = part if bacc is None else bacc + part
        bs.append(bacc)
    b = jnp.concatenate(bs, axis=1)
    assert st["staged"] == D
    a = jax.lax.dot_general(ot_scr[...].astype(BF16), wo_ref[...],
                            (((0,), (0,)), ((), ())),
                            preferred_element_type=F32)
    z = jnp.sum(xs.astype(F32) * gw_ref[...].astype(F32)[None, :],
                axis=-1, keepdims=True)
    g = jax.nn.sigmoid(z)
    o_ref[...] = (g * a + (1.0 - g) * b).astype(o_ref.dtype)


@jax.jit
def pallas_gated_mix__softmax_full_mha__dense_activation_relu__prompt_kernel(
    A_x: jax.Array,
    A_wqkv: jax.Array,
    A_wo: jax.Array,
    B_x: jax.Array,
    B_w1: jax.Array,
    B_w2: jax.Array,
    gate_w: jax.Array,
):
    del B_x
    out = pl.pallas_call(
        _kernel,
        grid=(NQ,),
        in_specs=[pl.BlockSpec(memory_space=pl.ANY)] * 6,
        out_specs=pl.BlockSpec((TQ, D), lambda i: (i, 0)),
        out_shape=jax.ShapeDtypeStruct((S, D), A_x.dtype),
        scratch_shapes=[
            pltpu.VMEM((S, D), BF16),
            pltpu.VMEM((3, D, D), BF16),
            pltpu.VMEM((D, D), BF16),
            pltpu.VMEM((D, DFF), BF16),
            pltpu.VMEM((DFF, D), BF16),
            pltpu.SemaphoreType.DMA((NR + 7,)),
            pltpu.VMEM((NWIN, S // 2, 128), U32),
            pltpu.VMEM((NR, D, OFFC, 128), F32),
            pltpu.VMEM((NQ, TQ // 128, D, 128), F32),
            pltpu.VMEM((D, 8, TQ), F32),
            pltpu.VMEM((NQ, H, 16, TQ), U32),
            pltpu.VMEM((NR, H, 24, TS), F32),
            pltpu.VMEM((S, 2 * TQ), F32),
            pltpu.VMEM((S, 2 * TQ), F32),
            pltpu.VMEM((2, 8, 2 * TQ), F32),
            pltpu.VMEM((D, TQ), F32),
            pltpu.VMEM((2 * OFFC, D), BF16),
            pltpu.VMEM((D,), BF16),
        ],
        compiler_params=pltpu.CompilerParams(
            dimension_semantics=("arbitrary",),
            vmem_limit_bytes=120 * 1024 * 1024,
        ),
    )(A_x.reshape(S, D), A_wqkv, A_wo, B_w1, B_w2, gate_w)
    return out.reshape(A_x.shape)
```
